```python
import os as _os
_os.environ.setdefault('JAX_PLATFORMS', 'cpu')
import jax
import jax.numpy as jnp

def _softmax(x, axis=-1):
    return jax.nn.softmax(x, axis=axis)

def _gelu(x):
    return jax.nn.gelu(x, approximate=True)

def _silu(x):
    return jax.nn.silu(x)

def _sigmoid(x):
    return jax.nn.sigmoid(x)

def _layernorm(x, axis=-1, eps=1e-05):
    m = jnp.mean(x, axis=axis, keepdims=True)
    v = jnp.var(x, axis=axis, keepdims=True)
    return (x - m) / jnp.sqrt(v + eps)

def _scatter_add(tgt, idx, src, axis=0):
    return tgt.at[idx].add(src)

def _segment_sum(src, seg, n):
    return jax.ops.segment_sum(src, seg, n)

class _Rng:

    def __init__(self, key):
        self._k = key

    def _next(self):
        self._k, sub = jax.random.split(self._k)
        return sub

    def normal(self, shape):
        return jax.random.normal(self._next(), shape, dtype=jnp.bfloat16)

    def randint(self, lo, hi, shape):
        return jax.random.randint(self._next(), shape, lo, hi, dtype=jnp.int32)

    def uniform(self, shape, lo=0.0, hi=1.0):
        return jax.random.uniform(self._next(), shape, jnp.bfloat16, lo, hi)

    def permutation(self, n):
        return jax.random.permutation(self._next(), n)
kernel_name = 'sequential_preLN__memory_aug_recurrent_mem_tr__swiglu_ffn__prompt'

def setup_inputs():
    _rng = _Rng(jax.random.key(int.from_bytes(__import__("os").urandom(4), "little")))
    _w = lambda a: (lambda t: t.astype(jnp.bfloat16) if jnp.issubdtype(t.dtype, jnp.floating) else t)(jnp.asarray(a))

    def _A_setup():
        B, S, Dm = (1, 2048, 640)
        H, Dh = (32, 192)
        M, seg = (8, 32)
        seg = min(seg, S)
        S = S // seg * seg
        return {'x': _w((lambda *s: _rng.normal(s) * 0.05)(B, S, Dm)), 'mem0': _w((lambda *s: _rng.normal(s) * 0.1)(B, M, Dm)), 'Wq': _w((lambda *s: _rng.normal(s) * 1.6)(Dm, H, Dh) * Dm ** (-0.5)), 'Wk': _w((lambda *s: _rng.normal(s) * 1.6)(Dm, H, Dh) * Dm ** (-0.5)), 'Wv': _w((lambda *s: _rng.normal(s) * 0.1)(Dm, H, Dh) * Dm ** (-0.5)), 'Wo': _w((lambda *s: _rng.normal(s) * 0.1)(H, Dh, Dm) * (H * Dh) ** (-0.5)), 'seg_len': seg}
    _A_in = _A_setup()

    def _B_setup():
        B, S, D, F = (1, 2048, 640, 1536)
        return {'x': _w((lambda *s: _rng.normal(s) * 0.05)(B, S, D)), 'w_gate': _w((lambda *s: _rng.normal(s) * 0.05)(D, F)), 'w_up': _w((lambda *s: _rng.normal(s) * 0.05)(D, F)), 'w_down': _w((lambda *s: _rng.normal(s) * 0.05)(F, D))}
    _B_in = _B_setup()
    return {'A_x': _A_in['x'], 'A_mem0': _A_in['mem0'], 'A_Wq': _A_in['Wq'], 'A_Wk': _A_in['Wk'], 'A_Wv': _A_in['Wv'], 'A_Wo': _A_in['Wo'], 'A_seg_len': _A_in['seg_len'], 'B_x': _B_in['x'], 'B_w_gate': _B_in['w_gate'], 'B_w_up': _B_in['w_up'], 'B_w_down': _B_in['w_down']}

def reference(A_x, A_mem0, A_Wq, A_Wk, A_Wv, A_Wo, A_seg_len, B_x, B_w_gate, B_w_up, B_w_down):

    def _A_ref(x, mem0, Wq, Wk, Wv, Wo, seg_len):
        B, S, Dm = x.shape
        H, Dh = (Wq.shape[1], Wq.shape[2])
        M = mem0.shape[1]
        scale = Dh ** (-0.5)
        n_seg = S // seg_len
        L = M + seg_len
        idx = jnp.arange(L)
        mask = (idx[:, None] < M) | (idx[:, None] >= idx[None, :])
        mem = mem0
        outs = []
        for s in range(n_seg):
            xs = x[:, s * seg_len:(s + 1) * seg_len, :].copy()
            h = jnp.concatenate([mem, xs], axis=1)
            q = jnp.einsum('btd,dhe->bhte', h, Wq)
            k = jnp.einsum('btd,dhe->bhte', h, Wk)
            v = jnp.einsum('btd,dhe->bhte', h, Wv)
            scores = jnp.einsum('bhqe,bhke->bhqk', q, k) * scale
            scores = jnp.where(mask[None, None], scores, -1000000000.0)
            p = _softmax(scores, axis=-1)
            o = jnp.einsum('bhqk,bhke->bhqe', p, v)
            o = jnp.einsum('bhte,hed->btd', o, Wo)
            mem = o[:, :M, :].copy()
            outs.append(o[:, M:, :])
        return jnp.concatenate(outs, axis=1)

    def _B_ref(x, w_gate, w_up, w_down):
        g = _silu(x @ w_gate)
        u = x @ w_up
        return g * u @ w_down
    x = A_x
    h = x + _A_ref(_layernorm(x, axis=-1), A_mem0, A_Wq, A_Wk, A_Wv, A_Wo, A_seg_len)
    h2 = h + _B_ref(_layernorm(h, axis=-1), B_w_gate, B_w_up, B_w_down)
    return h2
```

```python
import functools
import jax
import jax.numpy as jnp
from jax import lax
import jax.experimental.pallas as pl
import jax.experimental.pallas.tpu as pltpu

_NN = (((1,), (0,)), ((), ()))
_NT = (((1,), (1,)), ((), ()))
_EPS = 1e-5


def _dot(a, b, dims=_NN):
    return lax.dot_general(a, b, dims, preferred_element_type=jnp.float32)


def _ln(v):
    d = v.shape[-1]
    m = jnp.sum(v, axis=-1, keepdims=True) * (1.0 / d)
    c = v - m
    var = jnp.sum(c * c, axis=-1, keepdims=True) * (1.0 / d)
    return c * lax.rsqrt(var + _EPS)


NSLOT = 4
GR = 48
FC = 384


def _make_kernel(S, D, H, Dh, M, seg, F):
    L = M + seg
    NP = H // 2
    PW = 2 * Dh
    n_seg = S // seg
    scale = Dh ** (-0.5)
    TA = seg - M
    T0 = S - n_seg * TA
    R = 576
    C0 = R - T0
    LNB = (S - T0) // NP

    def kernel(x_hbm, mem0_ref, wq_hbm, wk_hbm, wv_hbm, wo_hbm, wg_hbm, wu_hbm, wd_hbm,
               out_hbm,
               x_v, xa_v, xb_v, out_v, stage, st_o, st_gu, st_d, st_x, wqkv, wo_v, wgu_v, wd_v,
               msc, ring_q, ring_k, ring_v,
               sem_w, sem_x, sem_o):
        srcs = (wq_hbm, wk_hbm, wv_hbm)
        rings = (ring_q, ring_k, ring_v)
        DR = F // NP

        def rows(p, n, base=0):
            return pl.ds(pl.multiple_of(base + p * n, 8), n)

        def gu_row(p):
            return jnp.minimum(p * GR, D - GR)

        def main_copies(p, slot):
            c = jnp.minimum(p, NP - 1)
            return [pltpu.make_async_copy(srcs[j].at[rows(c, PW)], stage.at[slot, pl.ds(j * PW, PW)],
                                          sem_w.at[slot, j]) for j in range(3)]

        def rest_copies(p, slot):
            c = jnp.minimum(p, NP - 1)
            gr = pl.ds(pl.multiple_of(gu_row(c), 16), GR)
            prs = ((x_hbm.at[rows(c, LNB, T0)], st_x.at[slot]),
                   (wo_hbm.at[rows(c, PW)], st_o.at[slot]),
                   (wd_hbm.at[rows(c, DR)], st_d.at[slot]),
                   (wg_hbm.at[gr], st_gu.at[slot, 0]),
                   (wu_hbm.at[gr], st_gu.at[slot, 1]))
            return [pltpu.make_async_copy(a, b, sem_w.at[slot, 3 + j]) for j, (a, b) in enumerate(prs)]

        x_a = pltpu.make_async_copy(x_hbm.at[pl.ds(0, T0)], x_v.at[pl.ds(0, T0)], sem_x)
        x_a.start()
        for c in main_copies(0, 0):
            c.start()
        x_a.wait()
        for c in rest_copies(0, 0) + main_copies(1, 1) + rest_copies(1, 1) + main_copies(2, 2):
            c.start()
        RB = 128

        def ln_body(i, _):
            xa_v[rows(i, RB), :] = _ln(x_v[rows(i, RB), :].astype(jnp.float32))
            return 0
        lax.fori_loop(0, T0 // RB, ln_body, 0)

        def pro_body(p, slots):
            slot, nxt, nxt2, nxt3 = slots
            for c in main_copies(p, slot) + rest_copies(p, slot):
                c.wait()
            def proj(j):
                rings[j][p, C0:R, :] = _dot(xa_v[...], stage[slot, j * PW:(j + 1) * PW, :], _NT)

            def flip(j):
                wqkv[p, :, j * PW:(j + 1) * PW] = pltpu.bitcast(stage[slot, j * PW:(j + 1) * PW, :].T, jnp.uint32)
            for c in rest_copies(p + 2, nxt2) + main_copies(p + 3, nxt3):
                c.start()
            proj(0)
            flip(0)
            flip(1)
            wo_v[rows(p, Dh), :] = pltpu.bitcast(st_o[slot], jnp.uint32)
            wd_v[rows(p, DR // 2), :] = pltpu.bitcast(st_d[slot], jnp.uint32)
            proj(1)
            flip(2)
            for j in range(2):
                wgu_v[rows(0, GR // 2, gu_row(p) // 2 + j * (D // 2)), :] = pltpu.bitcast(st_gu[slot, j], jnp.uint32)
            xs = st_x[slot]
            x_v[rows(p, LNB, T0), :] = xs
            xb_v[rows(p, LNB), :] = _ln(xs.astype(jnp.float32))
            proj(2)
            return nxt, nxt2, nxt3, slot
        lax.fori_loop(0, NP, pro_body, (jnp.int32(0), jnp.int32(1), jnp.int32(2), jnp.int32(3)))
        for c in rest_copies(NP, 0) + rest_copies(NP, 1) + main_copies(NP, 0) + main_copies(NP, 1) + main_copies(NP, 2):
            c.wait()
        bc = lambda t: pltpu.bitcast(t, jnp.bfloat16)

        row = lax.broadcasted_iota(jnp.int32, (L, 2 * L), 0)
        lane = lax.broadcasted_iota(jnp.int32, (L, 2 * L), 1)
        lo = lane < L
        key = jnp.where(lo, lane, lane - L)
        allow = (row < M) | (row >= key)
        first = lax.broadcasted_iota(jnp.int32, (L, 128), 1) < (Dh - 128)

        def ffn(s, att):
            r = pl.ds(pl.multiple_of(s * seg, seg), seg)
            h1 = x_v[r, :].astype(jnp.float32) + att
            hn = _ln(h1)
            g = _dot(hn, bc(wgu_v[0:D // 2, :]))
            u = _dot(hn, bc(wgu_v[D // 2:D, :]))
            a = g * jax.nn.sigmoid(g) * u
            out_v[r, :] = (h1 + _dot(a, bc(wd_v[...]))).astype(jnp.bfloat16)

        def out_copy(s):
            r = pl.ds(pl.multiple_of(s * seg, seg), seg)
            return pltpu.make_async_copy(out_v.at[r], out_hbm.at[r], sem_o)

        def blk(t):
            z = jnp.zeros((L, 128), jnp.float32)
            t1 = t[:, 128:256]
            top = jnp.concatenate([t[:, 0:128], jnp.where(first, t1, 0.0), z], axis=1)
            bot = jnp.concatenate([z, jnp.where(first, 0.0, t1), t[:, 256:384]], axis=1)
            return jnp.concatenate([top, bot], axis=0).astype(jnp.bfloat16)

        def softmax(sc):
            sc = jnp.where(allow, sc * scale, -1e9)
            m0 = jnp.max(jnp.where(lo, sc, -jnp.inf), axis=1, keepdims=True)
            m1 = jnp.max(jnp.where(lo, -jnp.inf, sc), axis=1, keepdims=True)
            e = jnp.exp(sc - jnp.where(lo, m0, m1))
            s0 = jnp.sum(jnp.where(lo, e, 0.0), axis=1, keepdims=True)
            s1 = jnp.sum(jnp.where(lo, 0.0, e), axis=1, keepdims=True)
            return e * jnp.where(lo, 1.0 / s0, 1.0 / s1)

        msc[0:M, :] = mem0_ref[...].astype(jnp.float32)
        msc[M:L, :] = jnp.zeros((seg, D), jnp.float32)

        def step(s, carry):
            wpos, rpos = carry
            prev = msc[M:L, :]
            h = jnp.concatenate([msc[0:M, :], xb_v[pl.ds(pl.multiple_of(s * TA, 8), TA), :]], axis=0)
            r = pl.ds(pl.multiple_of(jnp.maximum(s - 1, 0) * seg, seg), seg)
            wr = pl.ds(pl.multiple_of(wpos, 8), TA)
            rd = pl.ds(pl.multiple_of(rpos, 8), seg)
            h1 = x_v[r, :].astype(jnp.float32) + prev
            hn = _ln(h1)
            mq, pr, o = {}, {}, {}
            acc = None

            def part(p, j):
                return jnp.concatenate([mq[p, j], rings[j][p, rd, :]], axis=0)

            st = {}
            kw = dict(preferred_element_type=jnp.float32)

            def proj(p, j):
                t = lax.dot_general(h, bc(wqkv[p, :, j * PW:(j + 1) * PW]), _NN, **kw)
                mq[p, j] = t[0:M]
                rings[j][p, wr, :] = t[M:]

            def sc(p):
                pr[p] = softmax(lax.dot_general(part(p, 0), blk(part(p, 1)), _NT, **kw))

            def pv(p):
                o[p] = lax.dot_general(pr[p], blk(part(p, 2)), _NN, **kw)

            def outp(p, c):
                w = bc(wo_v[p * Dh + c * 64:p * Dh + (c + 1) * 64, :])
                d = lax.dot_general(o[p][:, c * 128:(c + 1) * 128], w, _NN, **kw)
                st['acc'] = st['acc'] + d if 'acc' in st else d

            def gate(c):
                st['g', c] = lax.dot_general(hn, bc(wgu_v[0:D // 2, c * FC:(c + 1) * FC]), _NN, **kw)

            def up(c):
                g = st['g', c]
                u = lax.dot_general(hn, bc(wgu_v[D // 2:D, c * FC:(c + 1) * FC]), _NN, **kw)
                st['a', c] = g * jax.nn.sigmoid(g) * u

            def down(c):
                d = lax.dot_general(st['a', c], bc(wd_v[c * FC // 2:(c + 1) * FC // 2, :]), _NN, **kw)
                st['y'] = st.get('y', h1) + d

            gu = [f for c in range(F // FC) for f in (functools.partial(gate, c), functools.partial(up, c))]
            outs = [functools.partial(outp, p, c) for p in range(NP) for c in range(3)]
            NH = 5
            lead = 10
            fill = [None] + [x for f in gu[:NH] for x in (f, None)][:lead - 1] + outs

            def run(fs):
                for f in fs:
                    if f is not None:
                        f()
            for i in range(NP):
                proj(i, 2)
                run(fill[3 * i:3 * i + 1])
                if i >= 1:
                    sc(i - 1)
                proj(i, 0)
                run(fill[3 * i + 1:3 * i + 2])
                proj(i, 1)
                run(fill[3 * i + 2:3 * i + 3])
                if i >= 2:
                    pv(i - 2)
            rest = fill[3 * NP:]
            gu = gu[NH:]
            run(rest[0:4])
            sc(NP - 1)
            pv(NP - 2)
            run(gu)
            pv(NP - 1)
            run(rest[4:7])
            down(0)
            down(1)
            run(rest[7:])
            down(2)
            down(3)
            out_v[r, :] = st['y'].astype(jnp.bfloat16)
            acc = st['acc']
            msc[...] = acc

            @pl.when(s > 0)
            def _():
                out_copy(s - 1).start()
            wpos = wpos + TA
            rpos = rpos + seg
            return (jnp.where(wpos >= R, wpos - R, wpos), jnp.where(rpos >= R, rpos - R, rpos))
        lax.fori_loop(0, n_seg, step, (jnp.int32(0), jnp.int32(C0)))
        ffn(n_seg - 1, msc[M:L, :])
        out_copy(n_seg - 1).start()
        pltpu.make_async_copy(out_v, out_hbm, sem_o).wait()

    return kernel, R, T0, LNB


@functools.partial(jax.jit, static_argnames=("A_seg_len",))
def pallas_sequential_preLN__memory_aug_recurrent_mem_tr__swiglu_ffn__prompt_kernel(
        A_x, A_mem0, A_Wq, A_Wk, A_Wv, A_Wo, A_seg_len, B_x, B_w_gate, B_w_up, B_w_down):
    B, S, D = A_x.shape
    H, Dh = A_Wq.shape[1], A_Wq.shape[2]
    M = A_mem0.shape[1]
    F = B_w_gate.shape[1]
    seg = int(A_seg_len)
    NP, PW = H // 2, 2 * Dh
    tr = lambda w: jnp.transpose(w, (1, 2, 0)).reshape(H * Dh, D)
    any_spec = pl.BlockSpec(memory_space=pl.ANY)
    bf = jnp.bfloat16
    u32 = jnp.uint32
    kern, R, T0, LNB = _make_kernel(S, D, H, Dh, M, seg, F)
    out = pl.pallas_call(
        kern,
        out_shape=jax.ShapeDtypeStruct((S, D), bf),
        in_specs=[any_spec, pl.BlockSpec(memory_space=pltpu.VMEM)] + [any_spec] * 7,
        out_specs=any_spec,
        scratch_shapes=[
            pltpu.VMEM((S, D), bf), pltpu.VMEM((T0, D), jnp.float32), pltpu.VMEM((S - T0, D), jnp.float32),
            pltpu.VMEM((S, D), bf),
            pltpu.VMEM((NSLOT, 3 * PW, D), bf), pltpu.VMEM((NSLOT, PW, D), bf),
            pltpu.VMEM((NSLOT, 2, GR, F), bf), pltpu.VMEM((NSLOT, F // NP, D), bf), pltpu.VMEM((NSLOT, LNB, D), bf),
            pltpu.VMEM((NP, D // 2, 3 * PW), u32), pltpu.VMEM((H * Dh // 2, D), u32),
            pltpu.VMEM((D, F), u32), pltpu.VMEM((F // 2, D), u32),
            pltpu.VMEM((M + seg, D), jnp.float32),
            pltpu.VMEM((NP, R, PW), jnp.float32), pltpu.VMEM((NP, R, PW), jnp.float32), pltpu.VMEM((NP, R, PW), jnp.float32),
            pltpu.SemaphoreType.DMA((NSLOT, 8)), pltpu.SemaphoreType.DMA, pltpu.SemaphoreType.DMA,
        ],
        compiler_params=pltpu.CompilerParams(vmem_limit_bytes=120 * 2**20),
    )(A_x.reshape(S, D), A_mem0.reshape(M, D), tr(A_Wq), tr(A_Wk), tr(A_Wv), A_Wo.reshape(H * Dh, D),
      B_w_gate, B_w_up, B_w_down)
    return out.reshape(B, S, D)
```

```python
import functools

import jax
import jax.numpy as jnp
from jax import lax
import jax.experimental.pallas as pl
import jax.experimental.pallas.tpu as pltpu

_NN = (((1,), (0,)), ((), ()))
_NT = (((1,), (1,)), ((), ()))
_EPS = 1e-5
_LANES = 128
_NSLOT = 4
_UNROLL = 4
_FC = 384
_GR = 48
_RSLOTS = 12


def _dot(a, b, dims=_NN):
    return lax.dot_general(a, b, dims, preferred_element_type=jnp.float32)


def _ln(v):
    d = v.shape[-1]
    m = jnp.sum(v, axis=-1, keepdims=True) * (1.0 / d)
    c = v - m
    var = jnp.sum(c * c, axis=-1, keepdims=True) * (1.0 / d)
    return c * lax.rsqrt(var + _EPS)


def _as_bf16(w):
    return pltpu.bitcast(w, jnp.bfloat16)


def _as_u32(w):
    return pltpu.bitcast(w, jnp.uint32)


def _build(S, D, H, Dh, M, seg, F):
    L = M + seg
    NP = H // 2
    PW = 2 * Dh
    n_seg = S // seg
    scale = Dh ** (-0.5)
    TA = seg - M
    T0 = S - n_seg * TA
    LNB = (S - T0) // NP
    DR = F // NP
    NR = 18
    C0 = NR - T0 // seg
    U = _UNROLL
    assert (M, seg, PW) == (8, 32, 3 * _LANES) and H % 2 == 0 and n_seg % U == 0
    assert T0 % _LANES == 0 and C0 >= 1 and NR % 3 == 0 and NP >= _NSLOT
    assert LNB % 16 == 0 and DR % 16 == 0 and NP * _GR >= D and D % 16 == 0 and F == 4 * _FC

    def kernel(x_hbm, mem0_hbm, wq_hbm, wk_hbm, wv_hbm, wo_hbm, wg_hbm, wu_hbm, wd_hbm,
               out_hbm,
               x_v, xa_v, xb_v, out_v, stage, st_o, st_gu, st_d, st_x,
               wqkv, wo_v, wgu_v, wd_v, ring_q, ring_k, ring_v, mem0_v, state_v,
               sem_w, sem_x, sem_0, sem_o):
        srcs = (wq_hbm, wk_hbm, wv_hbm)
        rings = (ring_q, ring_k, ring_v)

        def rows(p, n, base=0):
            return pl.ds(pl.multiple_of(base + p * n, 8), n)

        def gu_row(p):
            return jnp.minimum(p * _GR, D - _GR)

        def tile(p, g, c):
            return p * _RSLOTS + g * 3 + c

        def main_copies(p, slot):
            c = jnp.minimum(p, NP - 1)
            return [pltpu.make_async_copy(srcs[j].at[rows(c, PW)],
                                          stage.at[slot, pl.ds(j * PW, PW)],
                                          sem_w.at[slot, j]) for j in range(3)]

        def rest_copies(p, slot):
            c = jnp.minimum(p, NP - 1)
            gr = pl.ds(pl.multiple_of(gu_row(c), 16), _GR)
            pairs = ((x_hbm.at[rows(c, LNB, T0)], st_x.at[slot]),
                     (wo_hbm.at[rows(c, PW)], st_o.at[slot]),
                     (wd_hbm.at[rows(c, DR)], st_d.at[slot]),
                     (wg_hbm.at[gr], st_gu.at[slot, 0]),
                     (wu_hbm.at[gr], st_gu.at[slot, 1]))
            return [pltpu.make_async_copy(a, b, sem_w.at[slot, 3 + j])
                    for j, (a, b) in enumerate(pairs)]

        x_a = pltpu.make_async_copy(x_hbm.at[pl.ds(0, T0)], x_v.at[pl.ds(0, T0)], sem_x)
        m_0 = pltpu.make_async_copy(mem0_hbm, mem0_v, sem_0)
        x_a.start()
        for c in main_copies(0, 0):
            c.start()
        x_a.wait()
        m_0.start()
        for c in rest_copies(0, 0):
            c.start()

        def ln_body(i, _):
            xa_v[rows(i, _LANES), :] = _ln(x_v[rows(i, _LANES), :].astype(jnp.float32))
            return 0
        lax.fori_loop(0, T0 // _LANES, ln_body, 0)
        for c in main_copies(1, 1) + rest_copies(1, 1) + main_copies(2, 2):
            c.start()

        def pro_body(p, slots):
            slot, nxt, nxt2, nxt3 = slots
            for c in main_copies(p, slot) + rest_copies(p, slot):
                c.wait()
            for c in rest_copies(p + 2, nxt2) + main_copies(p + 3, nxt3):
                c.start()

            def proj(j):
                t = _dot(xa_v[...], stage[slot, j * PW:(j + 1) * PW, :], _NT)
                t = t.reshape(T0 // seg, seg // 8, 8, PW)
                for c in range(3):
                    for g in range(seg // 8):
                        rings[j][C0:NR, tile(p, g, c)] = t[:, g, :, c * _LANES:(c + 1) * _LANES]

            def flip(j):
                wqkv[p, :, j * PW:(j + 1) * PW] = _as_u32(stage[slot, j * PW:(j + 1) * PW, :].T)

            proj(0)
            flip(0)
            flip(1)
            wo_v[rows(p, Dh), :] = _as_u32(st_o[slot])
            wd_v[rows(p, DR // 2), :] = _as_u32(st_d[slot])
            proj(1)
            flip(2)
            for j in range(2):
                wgu_v[rows(0, _GR // 2, gu_row(p) // 2 + j * (D // 2)), :] = _as_u32(st_gu[slot, j])
            xs = st_x[slot]
            x_v[rows(p, LNB, T0), :] = xs
            xb_v[rows(p, LNB), :] = _ln(xs.astype(jnp.float32))
            proj(2)
            return nxt, nxt2, nxt3, slot
        lax.fori_loop(0, NP, pro_body, tuple(jnp.int32(i) for i in range(_NSLOT)))
        for i in range(2):
            for c in rest_copies(NP, (NP + i) % _NSLOT):
                c.wait()
        for i in range(3):
            for c in main_copies(NP, (NP + i) % _NSLOT):
                c.wait()

        row = lax.broadcasted_iota(jnp.int32, (L, 2 * L), 0)
        lane = lax.broadcasted_iota(jnp.int32, (L, 2 * L), 1)
        lo = lane < L
        key = jnp.where(lo, lane, lane - L)
        allow = (row < M) | (row >= key)
        first = lax.broadcasted_iota(jnp.int32, (L, _LANES), 1) < (Dh - _LANES)

        def blk(t):
            z = jnp.zeros((L, _LANES), jnp.float32)
            t0, t1, t2 = (t[:, c * _LANES:(c + 1) * _LANES] for c in range(3))
            top = jnp.concatenate([t0, jnp.where(first, t1, 0.0), z], axis=1)
            bot = jnp.concatenate([z, jnp.where(first, 0.0, t1), t2], axis=1)
            return jnp.concatenate([top, bot], axis=0).astype(jnp.bfloat16)

        def softmax(sc):
            sc = jnp.where(allow, sc * scale, -1e9)
            m0 = jnp.max(jnp.where(lo, sc, -jnp.inf), axis=1, keepdims=True)
            m1 = jnp.max(jnp.where(lo, -jnp.inf, sc), axis=1, keepdims=True)
            e = jnp.exp(sc - jnp.where(lo, m0, m1))
            s0 = jnp.sum(jnp.where(lo, e, 0.0), axis=1, keepdims=True)
            s1 = jnp.sum(jnp.where(lo, 0.0, e), axis=1, keepdims=True)
            return e * jnp.where(lo, 1.0 / s0, 1.0 / s1)

        def ffn_parts(s, att):
            r = pl.ds(pl.multiple_of(s * seg, seg), seg)
            h1 = x_v[r, :].astype(jnp.float32) + att
            hn = _ln(h1)
            st = {'y': h1}

            def gate(c):
                st['g', c] = _dot(hn, _as_bf16(wgu_v[0:D // 2, c * _FC:(c + 1) * _FC]))

            def up(c):
                g = st['g', c]
                u = _dot(hn, _as_bf16(wgu_v[D // 2:D, c * _FC:(c + 1) * _FC]))
                st['a', c] = g * jax.nn.sigmoid(g) * u

            def down(c):
                w = _as_bf16(wd_v[c * _FC // 2:(c + 1) * _FC // 2, :])
                st['y'] = st['y'] + _dot(st['a', c], w)

            def finish():
                out_v[r, :] = st['y'].astype(jnp.bfloat16)

            gu = [functools.partial(f, c) for c in range(F // _FC) for f in (gate, up)]
            return gu, [functools.partial(down, c) for c in range(F // _FC)], finish

        def step(s, n, wpos, rpos, state):
            ahead = xb_v[pl.ds(pl.multiple_of(s * TA, 8), TA), :]
            h = jnp.concatenate([state[0:M, :], ahead], axis=0)
            gu, downs, finish = ffn_parts(jnp.maximum(s - 1, 0), state[M:L, :])
            mem, pr, o, st = {}, {}, {}, {}

            def part(p, j):
                segs = [jnp.concatenate([rings[j][rpos, tile(p, g, c)] for c in range(3)], axis=1)
                        for g in range(seg // 8)]
                return jnp.concatenate([mem[p, j]] + segs, axis=0)

            def proj(p, j):
                t = _dot(h, _as_bf16(wqkv[p, :, j * PW:(j + 1) * PW]))
                mem[p, j] = t[0:M]
                for i in range(TA // 8):
                    hi, g = divmod((TA // 8) * n + i, seg // 8)
                    for c in range(3):
                        rings[j][wpos + hi, tile(p, g, c)] = (
                            t[M + 8 * i:M + 8 * i + 8, c * _LANES:(c + 1) * _LANES])

            def scores(p):
                pr[p] = softmax(_dot(part(p, 0), blk(part(p, 1)), _NT))

            def values(p):
                o[p] = _dot(pr[p], blk(part(p, 2)))

            def outp(p, c):
                w = _as_bf16(wo_v[p * Dh + c * 64:p * Dh + (c + 1) * 64, :])
                d = _dot(o[p][:, c * _LANES:(c + 1) * _LANES], w)
                st['acc'] = st['acc'] + d if 'acc' in st else d

            fill = [None] * 11 + [functools.partial(outp, p, c) for p in range(NP) for c in range(3)]
            for m in range(4):
                fill[2 + 2 * m] = gu[m]

            def filler():
                f = fill.pop(0)
                if f is not None:
                    f()

            for i in range(NP):
                proj(i, 2)
                filler()
                if i >= 1:
                    scores(i - 1)
                proj(i, 0)
                filler()
                proj(i, 1)
                filler()
                if i >= 2:
                    values(i - 2)
            todo = {'X': fill, 'G': gu[4:], 'D': downs,
                    'S': [functools.partial(scores, NP - 1)],
                    'P': [functools.partial(values, p) for p in (NP - 2, NP - 1)]}
            for ch in 'XXXXXSPGGGGXPXXDXDXDXD':
                todo[ch].pop(0)()
            assert not any(todo.values())
            finish()
            return st['acc']

        def out_copy(j):
            r = pl.ds(pl.multiple_of(j * U * seg, U * seg), U * seg)
            return pltpu.make_async_copy(out_v.at[r], out_hbm.at[r], sem_o)

        m_0.wait()
        state_v[0:M, :] = mem0_v[...].astype(jnp.float32)
        state_v[M:L, :] = jnp.zeros((seg, D), jnp.float32)

        def body(j, carry):
            wpos, rpos = carry
            state = state_v[...]
            for n in range(U):
                state = step(j * U + n, n, wpos, rpos, state)
                rpos = jnp.where(rpos + 1 >= NR, 0, rpos + 1)
            state_v[...] = state

            @pl.when(j > 0)
            def _():
                out_copy(j - 1).start()
            adv = U * TA // seg
            return jnp.where(wpos + adv >= NR, 0, wpos + adv), rpos
        lax.fori_loop(0, n_seg // U, body, (jnp.int32(0), jnp.int32(C0)))

        gu, downs, finish = ffn_parts(n_seg - 1, state_v[M:L, :])
        for f in gu + downs:
            f()
        finish()
        out_copy(n_seg // U - 1).start()
        pltpu.make_async_copy(out_v, out_hbm, sem_o).wait()

    bf, f32, u32 = jnp.bfloat16, jnp.float32, jnp.uint32
    ring = pltpu.VMEM((NR, NP * _RSLOTS, 8, _LANES), f32)
    scratch = [
        pltpu.VMEM((S, D), bf), pltpu.VMEM((T0, D), f32), pltpu.VMEM((S - T0, D), f32),
        pltpu.VMEM((S, D), bf),
        pltpu.VMEM((_NSLOT, 3 * PW, D), bf), pltpu.VMEM((_NSLOT, PW, D), bf),
        pltpu.VMEM((_NSLOT, 2, _GR, F), bf), pltpu.VMEM((_NSLOT, DR, D), bf),
        pltpu.VMEM((_NSLOT, LNB, D), bf),
        pltpu.VMEM((NP, D // 2, 3 * PW), u32), pltpu.VMEM((H * Dh // 2, D), u32),
        pltpu.VMEM((D, F), u32), pltpu.VMEM((F // 2, D), u32),
        ring, ring, ring,
        pltpu.VMEM((M, D), bf), pltpu.VMEM((L, D), f32),
        pltpu.SemaphoreType.DMA((_NSLOT, 8)), pltpu.SemaphoreType.DMA,
        pltpu.SemaphoreType.DMA, pltpu.SemaphoreType.DMA,
    ]
    return kernel, scratch


@functools.partial(jax.jit, static_argnames=("A_seg_len",))
def pallas_sequential_preLN__memory_aug_recurrent_mem_tr__swiglu_ffn__prompt_kernel(
        A_x, A_mem0, A_Wq, A_Wk, A_Wv, A_Wo, A_seg_len, B_x, B_w_gate, B_w_up, B_w_down):
    del B_x
    B, S, D = A_x.shape
    H, Dh = A_Wq.shape[1], A_Wq.shape[2]
    M = A_mem0.shape[1]
    F = B_w_gate.shape[1]
    assert B == 1
    kernel, scratch = _build(S, D, H, Dh, M, int(A_seg_len), F)

    def head_major(w):
        return jnp.transpose(w, (1, 2, 0)).reshape(H * Dh, D)

    any_spec = pl.BlockSpec(memory_space=pl.ANY)
    out = pl.pallas_call(
        kernel,
        out_shape=jax.ShapeDtypeStruct((S, D), jnp.bfloat16),
        in_specs=[any_spec] * 9,
        out_specs=any_spec,
        scratch_shapes=scratch,
        compiler_params=pltpu.CompilerParams(
            vmem_limit_bytes=112 * 2**20,
            flags={"XLA_TPU_EVENLY_DISTRIBUTE_CRITICAL_NODES": True}),
    )(A_x.reshape(S, D), A_mem0.reshape(M, D), head_major(A_Wq), head_major(A_Wk),
      head_major(A_Wv), A_Wo.reshape(H * Dh, D), B_w_gate, B_w_up, B_w_down)
    return out.reshape(B, S, D)
```
